```python
import jax
import jax.numpy as jnp

def _softmax(x, axis=-1):
    return jax.nn.softmax(x, axis=axis)

def _gelu(x):
    return jax.nn.gelu(x, approximate=True)

def _silu(x):
    return jax.nn.silu(x)

def _sigmoid(x):
    return jax.nn.sigmoid(x)

def _layernorm(x, axis=-1, eps=1e-05):
    m = jnp.mean(x, axis=axis, keepdims=True)
    v = jnp.var(x, axis=axis, keepdims=True)
    return (x - m) / jnp.sqrt(v + eps)

def _scatter_add(tgt, idx, src, axis=0):
    return tgt.at[idx].add(src)

def _segment_sum(src, seg, n):
    return jax.ops.segment_sum(src, seg, n)

class _Rng:

    def __init__(self, key):
        self._k = key

    def _next(self):
        self._k, sub = jax.random.split(self._k)
        return sub

    def normal(self, shape):
        return jax.random.normal(self._next(), shape, dtype=jnp.bfloat16)

    def randint(self, lo, hi, shape):
        return jax.random.randint(self._next(), shape, lo, hi, dtype=jnp.int32)

    def uniform(self, shape, lo=0.0, hi=1.0):
        return jax.random.uniform(self._next(), shape, jnp.bfloat16, lo, hi)

    def permutation(self, n):
        return jax.random.permutation(self._next(), n)
kernel_name = 'adaLN_cond__sliding_block_cached__mixer_gmlp__decode'

def setup_inputs():
    _rng = _Rng(jax.random.key(int.from_bytes(__import__("os").urandom(4), "little")))
    _w = lambda a: (lambda t: t.astype(jnp.bfloat16) if jnp.issubdtype(t.dtype, jnp.floating) else t)(jnp.asarray(a))

    def _A_setup():
        B, Sq, D = (1, 1, 448)
        Hq, Hkv, Sk, Dh = (16, 8, 65536, 256)
        assert Hq % Hkv == 0, (Hq, Hkv)
        return {'x': _w((lambda *s: _rng.normal(s) * 0.05)(B, Sq, D)), 'k_cache': _w((lambda *s: _rng.normal(s) * 0.05)(B, Hkv, Sk, Dh)), 'v_cache': _w((lambda *s: _rng.normal(s) * 0.05)(B, Hkv, Sk, Dh)), 'wq': _w((lambda *s: _rng.normal(s) * 0.05)(D, Hq * Dh) * D ** (-0.5)), 'wo': _w((lambda *s: _rng.normal(s) * 0.05)(Hq * Dh, D) * (Hq * Dh) ** (-0.5))}
    _A_in = _A_setup()

    def _B_setup():
        B, S, D, F = (1, 1, 448, 1792)
        Fh = F // 2
        return {'x': _w((lambda *s: _rng.normal(s) * 0.05)(B, S, D)), 'w_in': _w((lambda *s: _rng.normal(s) * 0.05)(D, 2 * Fh)), 'w_sp': _w(0.01 * (lambda *s: _rng.normal(s) * 0.05)(S, S)), 'b_sp': _w(1.0 + 0.01 * (lambda *s: _rng.normal(s) * 0.05)(S)), 'w_out': _w((lambda *s: _rng.normal(s) * 0.05)(Fh, D))}
    _B_in = _B_setup()
    return {'A_x': _A_in['x'], 'A_k_cache': _A_in['k_cache'], 'A_v_cache': _A_in['v_cache'], 'A_wq': _A_in['wq'], 'A_wo': _A_in['wo'], 'B_x': _B_in['x'], 'B_w_in': _B_in['w_in'], 'B_w_sp': _B_in['w_sp'], 'B_b_sp': _B_in['b_sp'], 'B_w_out': _B_in['w_out'], 'c': _w((lambda *s: _rng.normal(s) * 0.05)(1, 448)), 'w_mod': _w((lambda *s: _rng.normal(s) * 0.05)(448, 6 * 448) * 448 ** (-0.5))}

def reference(A_x, A_k_cache, A_v_cache, A_wq, A_wo, B_x, B_w_in, B_w_sp, B_b_sp, B_w_out, c, w_mod):

    def _A_ref(x, k_cache, v_cache, wq, wo):
        B, Sq, D = x.shape
        Hq, Dh = (16, 256)
        Hkv, Sk = (k_cache.shape[1], k_cache.shape[2])
        W = min(4096, max(256, Sk // 4))
        rep = Hq // Hkv
        q = (lambda x, *d: x.transpose(*d))((x @ wq).reshape(B, Sq, Hq, Dh), 0, 2, 1, 3)
        k = jnp.repeat(k_cache[:, :, Sk - W:, :], rep, axis=1)
        v = jnp.repeat(v_cache[:, :, Sk - W:, :], rep, axis=1)
        scores = jnp.einsum('bhqd,bhkd->bhqk', q, k) * Dh ** (-0.5)
        p = _softmax(scores, axis=-1)
        o = jnp.einsum('bhqk,bhkd->bhqd', p, v)
        return (lambda x, *d: x.transpose(*d))(o, 0, 2, 1, 3).reshape(B, Sq, Hq * Dh) @ wo

    def _B_ref(x, w_in, w_sp, b_sp, w_out):
        B, S, D = x.shape
        F = w_in.shape[-1]
        Fh = F // 2
        z = _gelu(jnp.einsum('bsd,df->bsf', x, w_in))
        z1 = z[..., :Fh].copy()
        z2 = _layernorm(z[..., Fh:], axis=-1)
        g = jnp.einsum('ts,bsf->btf', w_sp, z2) + b_sp[None, :, None]
        return jnp.einsum('bsf,fd->bsd', z1 * g, w_out)
    x = A_x
    mod = (_silu(c) @ w_mod).reshape(c.shape[0], 6, 1, -1)
    sa, ca, ga, sb, cb, gb = (mod[:, 0].copy(), mod[:, 1].copy(), mod[:, 2].copy(), mod[:, 3].copy(), mod[:, 4].copy(), mod[:, 5].copy())
    h = _layernorm(x, axis=-1) * (1 + ca) + sa
    x = x + ga * _A_ref(h, A_k_cache, A_v_cache, A_wq, A_wo)
    h = _layernorm(x, axis=-1) * (1 + cb) + sb
    x = x + gb * _B_ref(h, B_w_in, B_w_sp, B_b_sp, B_w_out)
    return x
```

```python
import functools

import jax
import jax.numpy as jnp
from jax import lax
from jax.experimental import pallas as pl
from jax.experimental.pallas import tpu as pltpu

D = 448
HQ = 16
HKV = 8
DH = 256
W = 4096
FH = 896
EPS = 1e-5
F32 = jnp.float32
BF16 = jnp.bfloat16
NT = (((1,), (1,)), ((), ()))


def _ln(x):
    m = jnp.mean(x, axis=-1, keepdims=True)
    d = x - m
    v = jnp.mean(d * d, axis=-1, keepdims=True)
    return d * lax.rsqrt(v + EPS)


class _Stream:
    def __init__(self, sems, window):
        self.sems = sems
        self.window = window
        self.pieces = []
        self.n_wait = 0
        self.n_start = 0

    def add(self, src, dst, prio):
        self.pieces.append((src, dst, prio))
        return len(self.pieces) - 1

    def _copy(self, i):
        src, dst, _ = self.pieces[i]
        return pltpu.make_async_copy(src, dst, self.sems.at[i % self.window])

    def _start_next(self):
        if self.n_start < len(self.pieces):
            self._copy(self.n_start).start(priority=self.pieces[self.n_start][2])
            self.n_start += 1

    def prime(self):
        while self.n_start < min(self.window, len(self.pieces)):
            self._start_next()

    def wait_through(self, idx):
        while self.n_wait <= idx:
            self._copy(self.n_wait).wait()
            self.n_wait += 1
            self._start_next()


def _kernel(x_hbm, c_hbm, wsp_hbm, bsp_hbm, k_hbm, v_hbm, wq_hbm, woT_hbm, win_hbm, woutT_hbm, wmod_hbm,
            o_ref,
            x_v, c_v, wsp_v, bsp_v, wmod_v, wq_v, k_v, v_v, woT_v, win_v, woutT_v, q_v, mod_v, sems, ssems,
            *, sk, window, r0, r1, wa, wb, win_pieces, wout_chunks, tail_prio):
    st = _Stream(sems, window)

    def add_rows(src, dst, n, a, b):
        r = 0
        last = None
        while r < n:
            for (m, p) in ((a, 0), (b, 1)):
                m = min(m, n - r)
                if m > 0:
                    last = st.add(src.at[pl.ds(r, m), :], dst.at[pl.ds(r, m), :], p)
                    r += m
        return last

    i_wmod = add_rows(wmod_hbm, wmod_v, D, wa, wb)
    i_wq = add_rows(wq_hbm, wq_v, D, wa, wb)
    i_wo = add_rows(woT_hbm, woT_v, D, wa, wb)
    pair = r0 + r1
    npair = W // pair
    kv_last = {}
    for j in range(HKV):
        for name, src, dst in (("k", k_hbm, k_v), ("v", v_hbm, v_v)):
            for p in range(npair):
                base = p * pair
                if r0 > 0:
                    st.add(src.at[0, j, pl.ds(sk - W + base, r0), :], dst.at[j, pl.ds(base, r0), :], 0)
                kv_last[name, j, p] = st.add(src.at[0, j, pl.ds(sk - W + base + r0, r1), :],
                                             dst.at[j, pl.ds(base + r0, r1), :], 1)
    rows = D // win_pieces
    for r in range(0, D, rows):
        i_win = st.add(win_hbm.at[pl.ds(r, rows), :], win_v.at[pl.ds(r, rows), :], tail_prio)
    i_wout = []
    r = 0
    for n in wout_chunks:
        i_wout.append((r, n, st.add(woutT_hbm.at[pl.ds(r, n), :], woutT_v.at[pl.ds(r, n), :], tail_prio)))
        r += n
    assert r == D

    st.prime()
    cp = pltpu.make_async_copy
    c_c = cp(c_hbm, c_v, ssems.at[0])
    c_x = cp(x_hbm, x_v, ssems.at[1])
    c_wsp = cp(wsp_hbm, wsp_v, ssems.at[2])
    c_bsp = cp(bsp_hbm, bsp_v, ssems.at[3])
    c_c.start()
    c_x.start()
    c_wsp.start()
    c_bsp.start()

    st.wait_through(i_wmod - 1)
    c_c.wait()
    cf = c_v[...].astype(F32)
    sc = (cf * jax.nn.sigmoid(cf)).astype(BF16)
    c_x.wait()
    x = jnp.broadcast_to(x_v[0].astype(F32), (8, D))
    lnx = _ln(x)
    st.wait_through(i_wmod)
    mod = jnp.dot(jnp.broadcast_to(sc, (8, D)), wmod_v[...], preferred_element_type=F32)
    for i in range(6):
        mod_v[i] = mod[:, i * D:(i + 1) * D]
    h = (lnx * (1.0 + mod_v[1]) + mod_v[0]).astype(BF16)
    st.wait_through(i_wq)
    q = jnp.dot(h, wq_v[...], preferred_element_type=F32) * (DH ** -0.5)
    row = lax.broadcasted_iota(jnp.int32, (8, DH), 0)
    for j in range(HKV):
        q_v[j] = jnp.where(row == 0, q[:, 2 * j * DH:(2 * j + 1) * DH], q[:, (2 * j + 1) * DH:(2 * j + 2) * DH])
    st.wait_through(i_wo)

    attn = jnp.zeros((8, D), F32)
    for j in range(HKV):
        qj = q_v[j].astype(BF16)
        s_parts = []
        for p in range(npair):
            st.wait_through(kv_last["k", j, p])
            s_parts.append(lax.dot_general(qj, k_v[j, p * pair:(p + 1) * pair, :], NT,
                                           preferred_element_type=F32))
        s = jnp.concatenate(s_parts, axis=1)
        m = jnp.max(s, axis=-1, keepdims=True)
        e = jnp.exp(s - m)
        l = jnp.sum(e, axis=-1, keepdims=True)
        pb = e.astype(BF16)
        acc = jnp.zeros((8, DH), F32)
        for p in range(npair):
            st.wait_through(kv_last["v", j, p])
            acc = acc + jnp.dot(pb[:, p * pair:(p + 1) * pair], v_v[j, p * pair:(p + 1) * pair, :],
                                preferred_element_type=F32)
        o = acc / l
        o0 = jnp.broadcast_to(o[0:1, :], (8, DH))
        o1 = jnp.broadcast_to(o[1:2, :], (8, DH))
        lhs = jnp.concatenate([o0, o1], axis=1).astype(BF16)
        attn = attn + lax.dot_general(lhs, woT_v[:, 2 * DH * j:2 * DH * (j + 1)], NT,
                                      preferred_element_type=F32)

    x1 = x + mod_v[2] * attn
    h2 = (_ln(x1) * (1.0 + mod_v[4]) + mod_v[3]).astype(BF16)
    c_wsp.wait()
    c_bsp.wait()
    wsp = wsp_v[...].astype(F32)
    bsp = bsp_v[...].astype(F32)
    st.wait_through(i_win)
    z = jnp.dot(h2, win_v[...], preferred_element_type=F32)
    z = jax.nn.gelu(z, approximate=True)
    z1 = z[:, :FH]
    z2 = _ln(z[:, FH:])
    g = z2 * wsp + bsp
    y = (z1 * g).astype(BF16)
    gb = mod_v[5]
    outs = []
    for (r, n, idx) in i_wout:
        st.wait_through(idx)
        outs.append(lax.dot_general(y, woutT_v[r:r + n, :], NT, preferred_element_type=F32))
    out = jnp.concatenate(outs, axis=1) if len(outs) > 1 else outs[0]
    x2 = x1 + gb * out
    o_ref[...] = x2[0:1, :].astype(BF16)


@jax.jit
def pallas_adaLN_cond__sliding_block_cached__mixer_gmlp__decode_kernel(
    A_x, A_k_cache, A_v_cache, A_wq, A_wo, B_x, B_w_in, B_w_sp, B_b_sp, B_w_out, c, w_mod,
):
    del B_x
    sk = A_k_cache.shape[2]
    window = 12
    any_spec = pl.BlockSpec(memory_space=pl.ANY)
    out = pl.pallas_call(
        functools.partial(_kernel, sk=sk, window=window, r0=128, r1=384, wa=8, wb=24,
                          win_pieces=4, wout_chunks=(128, 128, 128, 64), tail_prio=1),
        out_shape=jax.ShapeDtypeStruct((1, D), BF16),
        in_specs=[any_spec] * 11,
        out_specs=pl.BlockSpec(memory_space=pltpu.VMEM),
        scratch_shapes=[
            pltpu.VMEM((1, 1, D), BF16), pltpu.VMEM((1, D), BF16),
            pltpu.VMEM((1, 1), BF16), pltpu.VMEM((1, 1), BF16),
            pltpu.VMEM((D, 6 * D), BF16), pltpu.VMEM((D, HQ * DH), BF16),
            pltpu.VMEM((HKV, W, DH), BF16), pltpu.VMEM((HKV, W, DH), BF16),
            pltpu.VMEM((D, HQ * DH), BF16), pltpu.VMEM((D, 2 * FH), BF16), pltpu.VMEM((D, FH), BF16),
            pltpu.VMEM((HKV, 8, DH), F32), pltpu.VMEM((6, 8, D), F32),
            pltpu.SemaphoreType.DMA((window,)),
            pltpu.SemaphoreType.DMA((4,)),
        ],
        compiler_params=pltpu.CompilerParams(vmem_limit_bytes=100 * 1024 * 1024,
                                             disable_semaphore_checks=True),
    )(A_x, c, B_w_sp, B_b_sp.reshape(1, 1), A_k_cache, A_v_cache, A_wq, A_wo.T, B_w_in, B_w_out.T, w_mod)
    return out.reshape(1, 1, D)
```

```python
import functools

import jax
import jax.numpy as jnp
from jax import lax
from jax.experimental import pallas as pl
from jax.experimental.pallas import tpu as pltpu

D = 448
HQ = 16
HKV = 8
DH = 256
W = 4096
FH = 896
EPS = 1e-5
F32 = jnp.float32
BF16 = jnp.bfloat16
NT = (((1,), (1,)), ((), ()))


def _ln(x):
    m = jnp.mean(x, axis=-1, keepdims=True)
    d = x - m
    v = jnp.mean(d * d, axis=-1, keepdims=True)
    return d * lax.rsqrt(v + EPS)


class _Stream:
    def __init__(self, sems, nsem, window, group_units):
        self.sems = sems
        self.nsem = nsem
        self.window = window
        self.group_units = group_units
        self.units = []
        self.group_end = []
        self.n_wait = 0
        self.n_start = 0
        self._open = 0

    def add(self, small, bulk, close=False):
        self.units.append((small, bulk, len(self.group_end)))
        self._open += 1
        if close or self._open == self.group_units:
            self.close_group()
        return len(self.units) - 1

    def close_group(self):
        if self._open:
            self.group_end.append(len(self.units))
            self._open = 0

    def _copy(self, pair, group):
        return pltpu.make_async_copy(pair[0], pair[1], self.sems.at[group % self.nsem])

    def _can_start(self):
        if self.n_start >= len(self.units) or self.n_start - self.n_wait >= self.window:
            return False
        prev = self.units[self.n_start][2] - self.nsem
        return prev < 0 or self.group_end[prev] <= self.n_wait

    def _pump(self):
        while self._can_start():
            small, bulk, group = self.units[self.n_start]
            for pair in small:
                self._copy(pair, group).start(priority=0)
            self._copy(bulk, group).start(priority=1)
            self.n_start += 1

    def prime(self):
        self.close_group()
        self._pump()

    def wait_through(self, idx):
        end = self.group_end[self.units[idx][2]]
        while self.n_wait < end:
            group = self.units[self.n_wait][2]
            first = self.group_end[group - 1] if group else 0
            if self.n_wait == first:
                for u in range(first, self.group_end[group]):
                    for pair in self.units[u][0]:
                        self._copy(pair, group).wait()
            self._copy(self.units[self.n_wait][1], group).wait()
            self.n_wait += 1
            self._pump()


def _cuts(n, a, b):
    out = []
    r = 0
    while r < n:
        m = min(a + b, n - r)
        s = a if m > a else 0
        out.append((r, s, m - s))
        r += m
    return out


def _kernel(x_hbm, c_hbm, wsp_hbm, bsp_hbm, k_hbm, v_hbm, wq_hbm, woT_hbm, win_hbm, woutT_hbm, wmod_hbm,
            o_ref,
            x_v, c_v, wsp_v, bsp_v, wmod_v, wq_v, k_v, v_v, woT_v, win_v, woutT_v, q_v, mod_v, sems,
            *, sk, window, nsem, gsize, kv_pat, w_pat, chunk, win_pat, wout_cuts, wout_small):
    st = _Stream(sems, nsem, window, gsize)

    def add_rows(src, dst, n, a, b, extra=None, close_every=None):
        idx = []
        for (r, s, m) in _cuts(n, a, b):
            small = [(src.at[pl.ds(r, s), :], dst.at[pl.ds(r, s), :])] if s else []
            if extra and r == 0:
                small = small + extra
            bulk = (src.at[pl.ds(r + s, m), :], dst.at[pl.ds(r + s, m), :])
            end = r + s + m
            close = close_every is not None and (end % close_every == 0 or end == n)
            idx.append((r, end, st.add(small, bulk, close=close)))
        return idx

    def last_for(idx, end):
        return max(i for (r0, r1, i) in idx if r0 < end)

    wm_idx = add_rows(wmod_hbm, wmod_v, D, *w_pat,
                      extra=[(c_hbm, c_v), (x_hbm, x_v), (wsp_hbm, wsp_v), (bsp_hbm, bsp_v)])
    i_small, i_wmod = wm_idx[0][2], wm_idx[-1][2]
    i_wq = add_rows(wq_hbm, wq_v, D, *w_pat)[-1][2]
    i_wo = add_rows(woT_hbm, woT_v, D, *w_pat)[-1][2]
    kv = {}
    for j in range(HKV):
        kv["k", j] = add_rows(k_hbm.at[0, j, pl.ds(sk - W, W), :], k_v.at[j], W, *kv_pat)
        kv["v", j] = add_rows(v_hbm.at[0, j, pl.ds(sk - W, W), :], v_v.at[j], W, *kv_pat)
    st.close_group()
    win_idx = add_rows(win_hbm, win_v, D, *win_pat, close_every=128)
    wout_idx = []
    r = 0
    for n in wout_cuts:
        s = wout_small if n > wout_small else 0
        small = [(woutT_hbm.at[pl.ds(r, s), :], woutT_v.at[pl.ds(r, s), :])] if s else []
        wout_idx.append((r, r + n, st.add(small, (woutT_hbm.at[pl.ds(r + s, n - s), :],
                                                  woutT_v.at[pl.ds(r + s, n - s), :]), close=True)))
        r += n
    assert r == D

    st.prime()

    st.wait_through(i_small)
    cf = c_v[...].astype(F32)
    sc = (cf * jax.nn.sigmoid(cf)).astype(BF16)
    x = jnp.broadcast_to(x_v[0].astype(F32), (8, D))
    lnx = _ln(x)
    st.wait_through(i_wmod)
    mod = jnp.dot(jnp.broadcast_to(sc, (8, D)), wmod_v[...], preferred_element_type=F32)
    for i in range(6):
        mod_v[i] = mod[:, i * D:(i + 1) * D]
    h = (lnx * (1.0 + mod_v[1]) + mod_v[0]).astype(BF16)
    st.wait_through(i_wq)
    q = jnp.dot(h, wq_v[...], preferred_element_type=F32) * (DH ** -0.5)
    row = lax.broadcasted_iota(jnp.int32, (8, DH), 0)
    for j in range(HKV):
        q_v[j] = jnp.where(row == 0, q[:, 2 * j * DH:(2 * j + 1) * DH], q[:, (2 * j + 1) * DH:(2 * j + 2) * DH])
    st.wait_through(i_wo)

    attn = jnp.zeros((8, D), F32)
    nch = W // chunk
    for j in range(HKV):
        qj = q_v[j].astype(BF16)
        s_parts = []
        for p in range(nch):
            st.wait_through(last_for(kv["k", j], (p + 1) * chunk))
            s_parts.append(lax.dot_general(qj, k_v[j, p * chunk:(p + 1) * chunk, :], NT,
                                           preferred_element_type=F32))
        s = jnp.concatenate(s_parts, axis=1)
        m = jnp.max(s, axis=-1, keepdims=True)
        e = jnp.exp(s - m)
        l = jnp.sum(e, axis=-1, keepdims=True)
        pb = e.astype(BF16)
        acc = jnp.zeros((8, DH), F32)
        for p in range(nch):
            st.wait_through(last_for(kv["v", j], (p + 1) * chunk))
            acc = acc + jnp.dot(pb[:, p * chunk:(p + 1) * chunk], v_v[j, p * chunk:(p + 1) * chunk, :],
                                preferred_element_type=F32)
        o = acc / l
        o0 = jnp.broadcast_to(o[0:1, :], (8, DH))
        o1 = jnp.broadcast_to(o[1:2, :], (8, DH))
        lhs = jnp.concatenate([o0, o1], axis=1).astype(BF16)
        attn = attn + lax.dot_general(lhs, woT_v[:, 2 * DH * j:2 * DH * (j + 1)], NT,
                                      preferred_element_type=F32)

    x1 = x + mod_v[2] * attn
    h2 = (_ln(x1) * (1.0 + mod_v[4]) + mod_v[3]).astype(BF16)
    wsp = wsp_v[...].astype(F32)
    bsp = bsp_v[...].astype(F32)
    z = None
    for r0 in range(0, D, 128):
        r1 = min(r0 + 128, D)
        st.wait_through(last_for(win_idx, r1))
        part = jnp.dot(h2[:, r0:r1], win_v[r0:r1, :], preferred_element_type=F32)
        z = part if z is None else z + part
    z = jax.nn.gelu(z, approximate=True)
    z1 = z[:, :FH]
    z2 = _ln(z[:, FH:])
    g = z2 * wsp + bsp
    y = (z1 * g).astype(BF16)
    gb = mod_v[5]
    outs = []
    for (r0, r1, idx) in wout_idx:
        st.wait_through(idx)
        outs.append(lax.dot_general(y, woutT_v[r0:r1, :], NT, preferred_element_type=F32))
    out = jnp.concatenate(outs, axis=1) if len(outs) > 1 else outs[0]
    x2 = x1 + gb * out
    o_ref[...] = x2[0:1, :].astype(BF16)


@jax.jit
def pallas_adaLN_cond__sliding_block_cached__mixer_gmlp__decode_kernel(
    A_x, A_k_cache, A_v_cache, A_wq, A_wo, B_x, B_w_in, B_w_sp, B_b_sp, B_w_out, c, w_mod,
):
    del B_x
    sk = A_k_cache.shape[2]
    nsem = 4
    any_spec = pl.BlockSpec(memory_space=pl.ANY)
    out = pl.pallas_call(
        functools.partial(_kernel, sk=sk, window=12, nsem=nsem, gsize=4, kv_pat=(56, 168), w_pat=(8, 16),
                          chunk=256, win_pat=(0, 128), wout_cuts=(128, 128, 128, 64), wout_small=0),
        out_shape=jax.ShapeDtypeStruct((1, D), BF16),
        in_specs=[any_spec] * 11,
        out_specs=pl.BlockSpec(memory_space=pltpu.VMEM),
        scratch_shapes=[
            pltpu.VMEM((1, 1, D), BF16), pltpu.VMEM((1, D), BF16),
            pltpu.VMEM((1, 1), BF16), pltpu.VMEM((1, 1), BF16),
            pltpu.VMEM((D, 6 * D), BF16), pltpu.VMEM((D, HQ * DH), BF16),
            pltpu.VMEM((HKV, W, DH), BF16), pltpu.VMEM((HKV, W, DH), BF16),
            pltpu.VMEM((D, HQ * DH), BF16), pltpu.VMEM((D, 2 * FH), BF16), pltpu.VMEM((D, FH), BF16),
            pltpu.VMEM((HKV, 8, DH), F32), pltpu.VMEM((6, 8, D), F32),
            pltpu.SemaphoreType.DMA((nsem,)),
        ],
        compiler_params=pltpu.CompilerParams(vmem_limit_bytes=64 * 1024 * 1024),
    )(A_x, c, B_w_sp, B_b_sp.reshape(1, 1), A_k_cache, A_v_cache, A_wq, A_wo.T, B_w_in, B_w_out.T, w_mod)
    return out.reshape(1, 1, D)
```

```python
import functools

import jax
import jax.numpy as jnp
from jax import lax
from jax.experimental import pallas as pl
from jax.experimental.pallas import tpu as pltpu

D = 448
HQ = 16
HKV = 8
DH = 256
FH = 896
EPS = 1e-5
F32 = jnp.float32
BF16 = jnp.bfloat16
NT = (((1,), (1,)), ((), ()))


def _ln(x):
    m = jnp.mean(x, axis=-1, keepdims=True)
    d = x - m
    v = jnp.mean(d * d, axis=-1, keepdims=True)
    return d * lax.rsqrt(v + EPS)


class _Stream:
    def __init__(self, sems, nsem, window):
        self.sems, self.nsem, self.window = sems, nsem, window
        self.units = []
        self.n_copies = 0
        self.n_wait = 0
        self.n_start = 0

    def add(self, small, bulk):
        unit = []
        for pairs, prio in ((small, 0), (bulk, 1)):
            for src, dst in pairs:
                unit.append((src, dst, prio, self.n_copies % self.nsem))
                self.n_copies += 1
        self.units.append(unit)
        return len(self.units) - 1

    def _pump(self):
        while self.n_start < len(self.units) and self.n_start - self.n_wait < self.window:
            in_flight = sum(len(u) for u in self.units[self.n_wait:self.n_start + 1])
            assert in_flight <= self.nsem, (in_flight, self.nsem)
            for src, dst, prio, slot in self.units[self.n_start]:
                pltpu.make_async_copy(src, dst, self.sems.at[slot]).start(priority=prio)
            self.n_start += 1

    def prime(self):
        self._pump()

    def wait_through(self, idx):
        while self.n_wait <= idx:
            for src, dst, _, slot in self.units[self.n_wait]:
                pltpu.make_async_copy(src, dst, self.sems.at[slot]).wait()
            self.n_wait += 1
            self._pump()


def _tile_copies(src, dst, t0, t1):
    nct = src.shape[1] // 128
    out = []
    while t0 < t1:
        r, c = divmod(t0, nct)
        if c == 0 and t1 - t0 >= nct:
            nr = (t1 - t0) // nct
            rows, cols = pl.ds(8 * r, 8 * nr), pl.ds(0, 128 * nct)
            t0 += nr * nct
        else:
            nc = min(nct - c, t1 - t0)
            rows, cols = pl.ds(8 * r, 8), pl.ds(128 * c, 128 * nc)
            t0 += nc
        out.append((src.at[rows, cols], dst.at[rows, cols]))
    return out


def _add_rows(st, src, dst, r0, r1, small, bulk, even=False, extra=()):
    nct = src.shape[1] // 128
    t0, t1 = r0 // 8 * nct, r1 // 8 * nct
    if even:
        n = max(1, round((t1 - t0) / (small + bulk)))
        cuts = [t0 + (t1 - t0) * u // n for u in range(n + 1)]
    else:
        cuts = list(range(t0, t1, small + bulk)) + [t1]
    out = []
    for lo, hi in zip(cuts, cuts[1:]):
        s = small if hi - lo > small else 0
        u = st.add(_tile_copies(src, dst, lo, lo + s) + list(extra), _tile_copies(src, dst, lo + s, hi))
        extra = ()
        out.append((hi // nct * 8, u))
    return out


def _unit_for(ready, rows):
    return min(u for (r, u) in ready if r >= rows)


def _body(x_hbm, c_hbm, wsp_hbm, bsp_hbm, k_hbm, v_hbm, wq_hbm, woT_hbm, win_hbm, woutT_hbm, wmod_hbm,
          o_ref,
          x_v, c_v, wsp_v, bsp_v, wmod_v, wq_v, k_v, v_v, woT_v, win_v, woutT_v, q_v, mod_v, sems,
          *, sk, w, nsem, window, kv_pat, w_pat, win_pat, chunk, wout_cuts):
    st = _Stream(sems, nsem, window)
    small_inputs = [(c_hbm, c_v), (x_hbm, x_v), (wsp_hbm, wsp_v), (bsp_hbm, bsp_v)]
    u_wmod = _add_rows(st, wmod_hbm, wmod_v, 0, D, *w_pat, extra=small_inputs)
    u_wq = _add_rows(st, wq_hbm, wq_v, 0, D, *w_pat)
    u_wo = _add_rows(st, woT_hbm, woT_v, 0, D, *w_pat)
    u_k, u_v = [], []
    for j in range(HKV):
        rows = pl.ds(sk - w, w)
        u_k.append(_add_rows(st, k_hbm.at[0, j, rows, :], k_v.at[j], 0, w, *kv_pat))
        u_v.append(_add_rows(st, v_hbm.at[0, j, rows, :], v_v.at[j], 0, w, *kv_pat))
    u_win = [_add_rows(st, win_hbm, win_v, r, min(r + 128, D), *win_pat, even=True)[-1][1]
             for r in range(0, D, 128)]
    u_wout = []
    r = 0
    for n in wout_cuts:
        u_wout.append(_add_rows(st, woutT_hbm, woutT_v, r, r + n, 0, n * FH)[-1][1])
        r += n
    st.prime()

    st.wait_through(u_wmod[0][1])
    cf = c_v[...].astype(F32)
    sc = (cf * jax.nn.sigmoid(cf)).astype(BF16)
    x = jnp.broadcast_to(x_v[0].astype(F32), (8, D))
    lnx = _ln(x)
    st.wait_through(u_wmod[-1][1])
    mod = jnp.dot(jnp.broadcast_to(sc, (8, D)), wmod_v[...], preferred_element_type=F32)
    for i in range(6):
        mod_v[i] = mod[:, i * D:(i + 1) * D]
    h = (lnx * (1.0 + mod_v[1]) + mod_v[0]).astype(BF16)
    st.wait_through(u_wq[-1][1])
    q = jnp.dot(h, wq_v[...], preferred_element_type=F32) * (DH ** -0.5)
    row = lax.broadcasted_iota(jnp.int32, (8, DH), 0)
    for j in range(HKV):
        q_v[j] = jnp.where(row == 0, q[:, 2 * j * DH:(2 * j + 1) * DH], q[:, (2 * j + 1) * DH:(2 * j + 2) * DH])
    st.wait_through(u_wo[-1][1])

    attn = jnp.zeros((8, D), F32)
    nch = w // chunk
    for j in range(HKV):
        qj = q_v[j].astype(BF16)
        s_parts = []
        for p in range(nch):
            st.wait_through(_unit_for(u_k[j], (p + 1) * chunk))
            s_parts.append(lax.dot_general(qj, k_v[j, p * chunk:(p + 1) * chunk, :], NT,
                                           preferred_element_type=F32))
        s = jnp.concatenate(s_parts, axis=1)
        m = jnp.max(s, axis=-1, keepdims=True)
        e = jnp.exp(s - m)
        l = jnp.sum(e, axis=-1, keepdims=True)
        pb = e.astype(BF16)
        acc = jnp.zeros((8, DH), F32)
        for p in range(nch):
            st.wait_through(_unit_for(u_v[j], (p + 1) * chunk))
            acc = acc + jnp.dot(pb[:, p * chunk:(p + 1) * chunk], v_v[j, p * chunk:(p + 1) * chunk, :],
                                preferred_element_type=F32)
        o = acc / l
        o0 = jnp.broadcast_to(o[0:1, :], (8, DH))
        o1 = jnp.broadcast_to(o[1:2, :], (8, DH))
        lhs = jnp.concatenate([o0, o1], axis=1).astype(BF16)
        attn = attn + lax.dot_general(lhs, woT_v[:, 2 * DH * j:2 * DH * (j + 1)], NT,
                                      preferred_element_type=F32)

    x1 = x + mod_v[2] * attn
    h2 = (_ln(x1) * (1.0 + mod_v[4]) + mod_v[3]).astype(BF16)
    wsp = wsp_v[...].astype(F32)
    bsp = bsp_v[...].astype(F32)
    z = None
    for i, r0 in enumerate(range(0, D, 128)):
        r1 = min(r0 + 128, D)
        st.wait_through(u_win[i])
        part = jnp.dot(h2[:, r0:r1], win_v[r0:r1, :], preferred_element_type=F32)
        z = part if z is None else z + part
    z = jax.nn.gelu(z, approximate=True)
    z1 = z[:, :FH]
    z2 = _ln(z[:, FH:])
    g = z2 * wsp + bsp
    y = (z1 * g).astype(BF16)
    gb = mod_v[5]
    outs = []
    r = 0
    for n, u in zip(wout_cuts, u_wout):
        st.wait_through(u)
        outs.append(lax.dot_general(y, woutT_v[r:r + n, :], NT, preferred_element_type=F32))
        r += n
    out = jnp.concatenate(outs, axis=1)
    x2 = x1 + gb * out
    o_ref[...] = x2[0:1, :].astype(BF16)


def _kernel(*refs, nsem, **kw):
    pl.run_scoped(functools.partial(_body, *refs, nsem=nsem, **kw), pltpu.SemaphoreType.DMA((nsem,)))


@jax.jit
def pallas_adaLN_cond__sliding_block_cached__mixer_gmlp__decode_kernel(
    A_x, A_k_cache, A_v_cache, A_wq, A_wo, B_x, B_w_in, B_w_sp, B_b_sp, B_w_out, c, w_mod,
):
    del B_x
    sk = A_k_cache.shape[2]
    w = min(4096, max(256, sk // 4))
    any_spec = pl.BlockSpec(memory_space=pl.ANY)
    out = pl.pallas_call(
        functools.partial(_kernel, sk=sk, w=w, window=11, nsem=64, kv_pat=(14, 58), w_pat=(20, 60),
                          win_pat=(20, 60), chunk=256, wout_cuts=(128, 128, 128, 64)),
        out_shape=jax.ShapeDtypeStruct((1, D), BF16),
        in_specs=[any_spec] * 11,
        out_specs=pl.BlockSpec(memory_space=pltpu.VMEM),
        scratch_shapes=[
            pltpu.VMEM((1, 1, D), BF16), pltpu.VMEM((1, D), BF16),
            pltpu.VMEM((1, 1), BF16), pltpu.VMEM((1, 1), BF16),
            pltpu.VMEM((D, 6 * D), BF16), pltpu.VMEM((D, HQ * DH), BF16),
            pltpu.VMEM((HKV, w, DH), BF16), pltpu.VMEM((HKV, w, DH), BF16),
            pltpu.VMEM((D, HQ * DH), BF16), pltpu.VMEM((D, 2 * FH), BF16), pltpu.VMEM((D, FH), BF16),
            pltpu.VMEM((HKV, 8, DH), F32), pltpu.VMEM((6, 8, D), F32),
        ],
        compiler_params=pltpu.CompilerParams(vmem_limit_bytes=64 * 1024 * 1024),
    )(A_x, c, B_w_sp, B_b_sp.reshape(1, 1), A_k_cache, A_v_cache, A_wq, A_wo.T, B_w_in, B_w_out.T, w_mod)
    return out.reshape(1, 1, D)
```

```python
import functools

import jax
import jax.numpy as jnp
from jax import lax
from jax.experimental import pallas as pl
from jax.experimental.pallas import tpu as pltpu

D = 448
HQ = 16
HKV = 8
DH = 256
FH = 896
EPS = 1e-5
F32 = jnp.float32
BF16 = jnp.bfloat16
NT = (((1,), (1,)), ((), ()))

WINDOW = 11
NSEM = 64
KV_UNIT = (14, 58)
WEIGHT_UNIT = (20, 60)
KV_CHUNK = 256
WOUT_CUTS = (128, 128, 128, 64)


class _Stream:
    def __init__(self, sems):
        self.sems = sems
        self.units = []
        self.n_copies = 0
        self.n_wait = 0
        self.n_start = 0

    def add(self, small, bulk):
        unit = []
        for pairs, priority in ((small, 0), (bulk, 1)):
            for src, dst in pairs:
                unit.append((src, dst, priority, self.n_copies % NSEM))
                self.n_copies += 1
        self.units.append(unit)
        return len(self.units) - 1

    def pump(self):
        while self.n_start < len(self.units) and self.n_start - self.n_wait < WINDOW:
            in_flight = sum(len(u) for u in self.units[self.n_wait:self.n_start + 1])
            assert in_flight <= NSEM, (in_flight, NSEM)
            for src, dst, priority, slot in self.units[self.n_start]:
                pltpu.make_async_copy(src, dst, self.sems.at[slot]).start(priority=priority)
            self.n_start += 1

    def wait_through(self, idx):
        while self.n_wait <= idx:
            for src, dst, _, slot in self.units[self.n_wait]:
                pltpu.make_async_copy(src, dst, self.sems.at[slot]).wait()
            self.n_wait += 1
            self.pump()


def _tile_copies(src, dst, t0, t1):
    nct = src.shape[1] // 128
    out = []
    while t0 < t1:
        r, c = divmod(t0, nct)
        if c == 0 and t1 - t0 >= nct:
            nr = (t1 - t0) // nct
            rows, cols = pl.ds(8 * r, 8 * nr), pl.ds(0, 128 * nct)
            t0 += nr * nct
        else:
            nc = min(nct - c, t1 - t0)
            rows, cols = pl.ds(8 * r, 8), pl.ds(128 * c, 128 * nc)
            t0 += nc
        out.append((src.at[rows, cols], dst.at[rows, cols]))
    return out


def _add_rows(stream, src, dst, r0, r1, small, bulk, even=False, extra=()):
    nct = src.shape[1] // 128
    t0, t1 = r0 // 8 * nct, r1 // 8 * nct
    if even:
        n = max(1, round((t1 - t0) / (small + bulk)))
        cuts = [t0 + (t1 - t0) * u // n for u in range(n + 1)]
    else:
        cuts = list(range(t0, t1, small + bulk)) + [t1]
    out = []
    for lo, hi in zip(cuts, cuts[1:]):
        s = small if hi - lo > small else 0
        unit = stream.add(_tile_copies(src, dst, lo, lo + s) + list(extra),
                          _tile_copies(src, dst, lo + s, hi))
        extra = ()
        out.append((hi // nct * 8, unit))
    return out


def _unit_for(ready, rows):
    return min(unit for (done, unit) in ready if done >= rows)


def _layernorm(x):
    m = jnp.mean(x, axis=-1, keepdims=True)
    d = x - m
    v = jnp.mean(d * d, axis=-1, keepdims=True)
    return d * lax.rsqrt(v + EPS)


def _body(x_hbm, c_hbm, wsp_hbm, bsp_hbm, k_hbm, v_hbm, wq_hbm, woT_hbm, win_hbm, woutT_hbm, wmod_hbm,
          o_ref,
          x_v, c_v, wsp_v, bsp_v, wmod_v, wq_v, k_v, v_v, woT_v, win_v, woutT_v, q_v, mod_v,
          sems, *, sk, w):
    st = _Stream(sems)
    small_inputs = [(c_hbm, c_v), (x_hbm, x_v), (wsp_hbm, wsp_v), (bsp_hbm, bsp_v)]
    u_wmod = _add_rows(st, wmod_hbm, wmod_v, 0, D, *WEIGHT_UNIT, extra=small_inputs)
    u_wq = _add_rows(st, wq_hbm, wq_v, 0, D, *WEIGHT_UNIT)
    u_wo = _add_rows(st, woT_hbm, woT_v, 0, D, *WEIGHT_UNIT)
    u_k, u_v = [], []
    for j in range(HKV):
        window = pl.ds(sk - w, w)
        u_k.append(_add_rows(st, k_hbm.at[0, j, window, :], k_v.at[j], 0, w, *KV_UNIT))
        u_v.append(_add_rows(st, v_hbm.at[0, j, window, :], v_v.at[j], 0, w, *KV_UNIT))
    win_cuts = list(range(0, D, 128)) + [D]
    u_win = [_add_rows(st, win_hbm, win_v, r0, r1, *WEIGHT_UNIT, even=True)[-1][1]
             for r0, r1 in zip(win_cuts, win_cuts[1:])]
    wout_cuts = [sum(WOUT_CUTS[:i]) for i in range(len(WOUT_CUTS) + 1)]
    u_wout = [_add_rows(st, woutT_hbm, woutT_v, r0, r1, 0, (r1 - r0) * FH)[-1][1]
              for r0, r1 in zip(wout_cuts, wout_cuts[1:])]
    st.pump()

    st.wait_through(u_wmod[0][1])
    cf = c_v[...].astype(F32)
    sc = (cf * jax.nn.sigmoid(cf)).astype(BF16)
    x = jnp.broadcast_to(x_v[0].astype(F32), (8, D))
    lnx = _layernorm(x)
    st.wait_through(u_wmod[-1][1])
    mod = jnp.dot(jnp.broadcast_to(sc, (8, D)), wmod_v[...], preferred_element_type=F32)
    for i in range(6):
        mod_v[i] = mod[:, i * D:(i + 1) * D]

    h = (lnx * (1.0 + mod_v[1]) + mod_v[0]).astype(BF16)
    st.wait_through(u_wq[-1][1])
    q = jnp.dot(h, wq_v[...], preferred_element_type=F32) * (DH ** -0.5)
    row = lax.broadcasted_iota(jnp.int32, (8, DH), 0)
    for j in range(HKV):
        q_v[j] = jnp.where(row == 0, q[:, 2 * j * DH:(2 * j + 1) * DH],
                           q[:, (2 * j + 1) * DH:(2 * j + 2) * DH])
    st.wait_through(u_wo[-1][1])

    attn = jnp.zeros((8, D), F32)
    chunks = [(r, r + KV_CHUNK) for r in range(0, w, KV_CHUNK)]
    for j in range(HKV):
        qj = q_v[j].astype(BF16)
        scores = []
        for r0, r1 in chunks:
            st.wait_through(_unit_for(u_k[j], r1))
            scores.append(lax.dot_general(qj, k_v[j, r0:r1, :], NT, preferred_element_type=F32))
        s = jnp.concatenate(scores, axis=1)
        e = jnp.exp(s - jnp.max(s, axis=-1, keepdims=True))
        denom = jnp.sum(e, axis=-1, keepdims=True)
        p = e.astype(BF16)
        acc = jnp.zeros((8, DH), F32)
        for r0, r1 in chunks:
            st.wait_through(_unit_for(u_v[j], r1))
            acc = acc + jnp.dot(p[:, r0:r1], v_v[j, r0:r1, :], preferred_element_type=F32)
        o = acc / denom
        o_pair = jnp.concatenate([jnp.broadcast_to(o[0:1, :], (8, DH)),
                                  jnp.broadcast_to(o[1:2, :], (8, DH))], axis=1).astype(BF16)
        attn = attn + lax.dot_general(o_pair, woT_v[:, 2 * DH * j:2 * DH * (j + 1)], NT,
                                      preferred_element_type=F32)

    x1 = x + mod_v[2] * attn
    h2 = (_layernorm(x1) * (1.0 + mod_v[4]) + mod_v[3]).astype(BF16)
    z = None
    for (r0, r1), unit in zip(zip(win_cuts, win_cuts[1:]), u_win):
        st.wait_through(unit)
        part = jnp.dot(h2[:, r0:r1], win_v[r0:r1, :], preferred_element_type=F32)
        z = part if z is None else z + part
    z = jax.nn.gelu(z, approximate=True)
    g = _layernorm(z[:, FH:]) * wsp_v[...].astype(F32) + bsp_v[...].astype(F32)
    y = (z[:, :FH] * g).astype(BF16)
    outs = []
    for (r0, r1), unit in zip(zip(wout_cuts, wout_cuts[1:]), u_wout):
        st.wait_through(unit)
        outs.append(lax.dot_general(y, woutT_v[r0:r1, :], NT, preferred_element_type=F32))
    x2 = x1 + mod_v[5] * jnp.concatenate(outs, axis=1)
    o_ref[...] = x2[0:1, :].astype(BF16)


def _kernel(*refs, **kwargs):
    pl.run_scoped(functools.partial(_body, *refs, **kwargs), pltpu.SemaphoreType.DMA((NSEM,)))


@jax.jit
def pallas_adaLN_cond__sliding_block_cached__mixer_gmlp__decode_kernel(
    A_x: jax.Array,
    A_k_cache: jax.Array,
    A_v_cache: jax.Array,
    A_wq: jax.Array,
    A_wo: jax.Array,
    B_x: jax.Array,
    B_w_in: jax.Array,
    B_w_sp: jax.Array,
    B_b_sp: jax.Array,
    B_w_out: jax.Array,
    c: jax.Array,
    w_mod: jax.Array,
):
    del B_x
    sk = A_k_cache.shape[2]
    w = min(4096, max(256, sk // 4))
    any_spec = pl.BlockSpec(memory_space=pl.ANY)
    out = pl.pallas_call(
        functools.partial(_kernel, sk=sk, w=w),
        out_shape=jax.ShapeDtypeStruct((1, D), BF16),
        in_specs=[any_spec] * 11,
        out_specs=pl.BlockSpec(memory_space=pltpu.VMEM),
        scratch_shapes=[
            pltpu.VMEM((1, 1, D), BF16),
            pltpu.VMEM((1, D), BF16),
            pltpu.VMEM((1, 1), BF16),
            pltpu.VMEM((1, 1), BF16),
            pltpu.VMEM((D, 6 * D), BF16),
            pltpu.VMEM((D, HQ * DH), BF16),
            pltpu.VMEM((HKV, w, DH), BF16),
            pltpu.VMEM((HKV, w, DH), BF16),
            pltpu.VMEM((D, HQ * DH), BF16),
            pltpu.VMEM((D, 2 * FH), BF16),
            pltpu.VMEM((D, FH), BF16),
            pltpu.VMEM((HKV, 8, DH), F32),
            pltpu.VMEM((6, 8, D), F32),
        ],
        compiler_params=pltpu.CompilerParams(vmem_limit_bytes=64 * 1024 * 1024),
    )(A_x, c, B_w_sp, B_b_sp.reshape(1, 1), A_k_cache, A_v_cache, A_wq, A_wo.T, B_w_in, B_w_out.T,
      w_mod)
    return out.reshape(1, 1, D)
```

```python
import functools

import jax
import jax.numpy as jnp
from jax import lax
from jax.experimental import pallas as pl
from jax.experimental.pallas import tpu as pltpu

D = 448
HQ = 16
HKV = 8
DH = 256
FH = 896
EPS = 1e-5
F32 = jnp.float32
BF16 = jnp.bfloat16
NT = (((1,), (1,)), ((), ()))

WINDOW = 10
NSEM = 96
KV_UNIT = (48, 48)
WMOD_UNIT = (16, 48)
WQO_UNIT = (16, 80)
WIN_UNIT = (32, 48)
KV_CHUNK = 128
WOUT_CUTS = (128, 128, 128, 64)


class _Stream:
    def __init__(self, sems):
        self.sems = sems
        self.units = []
        self.n_copies = 0
        self.n_wait = 0
        self.n_start = 0

    def add(self, small, bulk):
        unit = []
        for pairs, priority in ((small, 0), (bulk, 1)):
            for src, dst in pairs:
                unit.append((src, dst, priority, self.n_copies % NSEM))
                self.n_copies += 1
        self.units.append(unit)
        return len(self.units) - 1

    def pump(self):
        while self.n_start < len(self.units) and self.n_start - self.n_wait < WINDOW:
            in_flight = sum(len(u) for u in self.units[self.n_wait:self.n_start + 1])
            assert in_flight <= NSEM, (in_flight, NSEM)
            for src, dst, priority, slot in self.units[self.n_start]:
                pltpu.make_async_copy(src, dst, self.sems.at[slot]).start(priority=priority)
            self.n_start += 1

    def wait_through(self, idx):
        while self.n_wait <= idx:
            for src, dst, _, slot in self.units[self.n_wait]:
                pltpu.make_async_copy(src, dst, self.sems.at[slot]).wait()
            self.n_wait += 1
            self.pump()


def _tile_copies(src, dst, t0, t1):
    nct = src.shape[1] // 128
    out = []
    while t0 < t1:
        r, c = divmod(t0, nct)
        if c == 0 and t1 - t0 >= nct:
            nr = (t1 - t0) // nct
            rows, cols = pl.ds(8 * r, 8 * nr), pl.ds(0, 128 * nct)
            t0 += nr * nct
        else:
            nc = min(nct - c, t1 - t0)
            rows, cols = pl.ds(8 * r, 8), pl.ds(128 * c, 128 * nc)
            t0 += nc
        out.append((src.at[rows, cols], dst.at[rows, cols]))
    return out


def _add_rows(stream, src, dst, r0, r1, small, bulk, even=False, extra=()):
    nct = src.shape[1] // 128
    t0, t1 = r0 // 8 * nct, r1 // 8 * nct
    if even:
        n = max(1, round((t1 - t0) / (small + bulk)))
        cuts = [t0 + (t1 - t0) * u // n for u in range(n + 1)]
    else:
        cuts = list(range(t0, t1, small + bulk)) + [t1]
    out = []
    for lo, hi in zip(cuts, cuts[1:]):
        s = small if hi - lo > small else 0
        unit = stream.add(_tile_copies(src, dst, lo, lo + s) + list(extra),
                          _tile_copies(src, dst, lo + s, hi))
        extra = ()
        out.append((hi // nct * 8, unit))
    return out


def _unit_for(ready, rows):
    return min(unit for (done, unit) in ready if done >= rows)


def _layernorm(x):
    m = jnp.mean(x, axis=-1, keepdims=True)
    d = x - m
    v = jnp.mean(d * d, axis=-1, keepdims=True)
    return d * lax.rsqrt(v + EPS)


def _body(x_hbm, c_hbm, wsp_hbm, bsp_hbm, k_hbm, v_hbm, wq_hbm, woT_hbm, win_hbm, woutT_hbm, wmod_hbm,
          o_ref,
          x_v, c_v, wsp_v, bsp_v, wmod_v, wq_v, k_v, v_v, woT_v, win_v, woutT_v, q_v, mod_v,
          sems, *, sk, w):
    st = _Stream(sems)
    small_inputs = [(c_hbm, c_v), (x_hbm, x_v), (wsp_hbm, wsp_v), (bsp_hbm, bsp_v)]
    u_wmod = _add_rows(st, wmod_hbm, wmod_v, 0, D, *WMOD_UNIT, extra=small_inputs)
    u_wq = _add_rows(st, wq_hbm, wq_v, 0, D, *WQO_UNIT)
    u_wo = _add_rows(st, woT_hbm, woT_v, 0, D, *WQO_UNIT)
    u_k, u_v = [], []
    for j in range(HKV):
        window = pl.ds(sk - w, w)
        u_k.append(_add_rows(st, k_hbm.at[0, j, window, :], k_v.at[j], 0, w, *KV_UNIT))
        u_v.append(_add_rows(st, v_hbm.at[0, j, window, :], v_v.at[j], 0, w, *KV_UNIT))
    win_cuts = list(range(0, D, 128)) + [D]
    u_win = [_add_rows(st, win_hbm, win_v, r0, r1, *WIN_UNIT, even=True)[-1][1]
             for r0, r1 in zip(win_cuts, win_cuts[1:])]
    wout_cuts = [sum(WOUT_CUTS[:i]) for i in range(len(WOUT_CUTS) + 1)]
    u_wout = [_add_rows(st, woutT_hbm, woutT_v, r0, r1, 0, (r1 - r0) * FH)[-1][1]
              for r0, r1 in zip(wout_cuts, wout_cuts[1:])]
    st.pump()

    st.wait_through(u_wmod[0][1])
    cf = c_v[...].astype(F32)
    sc = (cf * jax.nn.sigmoid(cf)).astype(BF16)
    x = jnp.broadcast_to(x_v[0].astype(F32), (8, D))
    lnx = _layernorm(x)
    st.wait_through(u_wmod[-1][1])
    mod = jnp.dot(jnp.broadcast_to(sc, (8, D)), wmod_v[...], preferred_element_type=F32)
    for i in range(6):
        mod_v[i] = mod[:, i * D:(i + 1) * D]

    h = (lnx * (1.0 + mod_v[1]) + mod_v[0]).astype(BF16)
    st.wait_through(u_wq[-1][1])
    q = jnp.dot(h, wq_v[...], preferred_element_type=F32) * (DH ** -0.5)
    row = lax.broadcasted_iota(jnp.int32, (8, DH), 0)
    for j in range(HKV):
        q_v[j] = jnp.where(row == 0, q[:, 2 * j * DH:(2 * j + 1) * DH],
                           q[:, (2 * j + 1) * DH:(2 * j + 2) * DH])
    st.wait_through(u_wo[-1][1])

    attn = jnp.zeros((8, D), F32)
    chunks = [(r, r + KV_CHUNK) for r in range(0, w, KV_CHUNK)]
    for j in range(HKV):
        qj = q_v[j].astype(BF16)
        scores = []
        for r0, r1 in chunks:
            st.wait_through(_unit_for(u_k[j], r1))
            scores.append(lax.dot_general(qj, k_v[j, r0:r1, :], NT, preferred_element_type=F32))
        s = jnp.concatenate(scores, axis=1)
        e = jnp.exp(s - jnp.max(s, axis=-1, keepdims=True))
        denom = jnp.sum(e, axis=-1, keepdims=True)
        p = e.astype(BF16)
        acc = jnp.zeros((8, DH), F32)
        for r0, r1 in chunks:
            st.wait_through(_unit_for(u_v[j], r1))
            acc = acc + jnp.dot(p[:, r0:r1], v_v[j, r0:r1, :], preferred_element_type=F32)
        o = acc / denom
        o_pair = jnp.concatenate([jnp.broadcast_to(o[0:1, :], (8, DH)),
                                  jnp.broadcast_to(o[1:2, :], (8, DH))], axis=1).astype(BF16)
        attn = attn + lax.dot_general(o_pair, woT_v[:, 2 * DH * j:2 * DH * (j + 1)], NT,
                                      preferred_element_type=F32)

    x1 = x + mod_v[2] * attn
    h2 = (_layernorm(x1) * (1.0 + mod_v[4]) + mod_v[3]).astype(BF16)
    z = None
    for (r0, r1), unit in zip(zip(win_cuts, win_cuts[1:]), u_win):
        st.wait_through(unit)
        part = jnp.dot(h2[:, r0:r1], win_v[r0:r1, :], preferred_element_type=F32)
        z = part if z is None else z + part
    z = jax.nn.gelu(z, approximate=True)
    g = _layernorm(z[:, FH:]) * wsp_v[...].astype(F32) + bsp_v[...].astype(F32)
    y = (z[:, :FH] * g).astype(BF16)
    outs = []
    for (r0, r1), unit in zip(zip(wout_cuts, wout_cuts[1:]), u_wout):
        st.wait_through(unit)
        outs.append(lax.dot_general(y, woutT_v[r0:r1, :], NT, preferred_element_type=F32))
    x2 = x1 + mod_v[5] * jnp.concatenate(outs, axis=1)
    o_ref[...] = x2[0:1, :].astype(BF16)


def _kernel(*refs, **kwargs):
    pl.run_scoped(functools.partial(_body, *refs, **kwargs), pltpu.SemaphoreType.DMA((NSEM,)))


@jax.jit
def pallas_adaLN_cond__sliding_block_cached__mixer_gmlp__decode_kernel(
    A_x: jax.Array,
    A_k_cache: jax.Array,
    A_v_cache: jax.Array,
    A_wq: jax.Array,
    A_wo: jax.Array,
    B_x: jax.Array,
    B_w_in: jax.Array,
    B_w_sp: jax.Array,
    B_b_sp: jax.Array,
    B_w_out: jax.Array,
    c: jax.Array,
    w_mod: jax.Array,
):
    del B_x
    sk = A_k_cache.shape[2]
    w = min(4096, max(256, sk // 4))
    any_spec = pl.BlockSpec(memory_space=pl.ANY)
    out = pl.pallas_call(
        functools.partial(_kernel, sk=sk, w=w),
        out_shape=jax.ShapeDtypeStruct((1, D), BF16),
        in_specs=[any_spec] * 11,
        out_specs=pl.BlockSpec(memory_space=pltpu.VMEM),
        scratch_shapes=[
            pltpu.VMEM((1, 1, D), BF16),
            pltpu.VMEM((1, D), BF16),
            pltpu.VMEM((1, 1), BF16),
            pltpu.VMEM((1, 1), BF16),
            pltpu.VMEM((D, 6 * D), BF16),
            pltpu.VMEM((D, HQ * DH), BF16),
            pltpu.VMEM((HKV, w, DH), BF16),
            pltpu.VMEM((HKV, w, DH), BF16),
            pltpu.VMEM((D, HQ * DH), BF16),
            pltpu.VMEM((D, 2 * FH), BF16),
            pltpu.VMEM((D, FH), BF16),
            pltpu.VMEM((HKV, 8, DH), F32),
            pltpu.VMEM((6, 8, D), F32),
        ],
        compiler_params=pltpu.CompilerParams(vmem_limit_bytes=64 * 1024 * 1024),
    )(A_x, c, B_w_sp, B_b_sp.reshape(1, 1), A_k_cache, A_v_cache, A_wq, A_wo.T, B_w_in, B_w_out.T,
      w_mod)
    return out.reshape(1, 1, D)
```

```python
import functools

import jax
import jax.numpy as jnp
from jax import lax
from jax.experimental import pallas as pl
from jax.experimental.pallas import tpu as pltpu

D = 448
HQ = 16
HKV = 8
DH = 256
FH = 896
EPS = 1e-5
F32 = jnp.float32
BF16 = jnp.bfloat16
NT = (((1,), (1,)), ((), ()))

WINDOW = 13
NSEM = 128
UNIT = (24, 48)
KV_CHUNK = 128
WOUT_CUTS = (128, 128, 128, 64)


class _Stream:
    def __init__(self, sems):
        self.sems = sems
        self.units = []
        self.n_copies = 0
        self.n_wait = 0
        self.n_start = 0

    def add(self, small, bulk):
        unit = []
        for pairs, priority in ((small, 0), (bulk, 1)):
            for src, dst in pairs:
                unit.append((src, dst, priority, self.n_copies % NSEM))
                self.n_copies += 1
        self.units.append(unit)
        return len(self.units) - 1

    def pump(self):
        while self.n_start < len(self.units) and self.n_start - self.n_wait < WINDOW:
            in_flight = sum(len(u) for u in self.units[self.n_wait:self.n_start + 1])
            assert in_flight <= NSEM, (in_flight, NSEM)
            for src, dst, priority, slot in self.units[self.n_start]:
                pltpu.make_async_copy(src, dst, self.sems.at[slot]).start(priority=priority)
            self.n_start += 1

    def wait_through(self, idx):
        while self.n_wait <= idx:
            for src, dst, _, slot in self.units[self.n_wait]:
                pltpu.make_async_copy(src, dst, self.sems.at[slot]).wait()
            self.n_wait += 1
            self.pump()


def _tile_copies(src, dst, t0, t1):
    nct = src.shape[1] // 128
    out = []
    while t0 < t1:
        r, c = divmod(t0, nct)
        if c == 0 and t1 - t0 >= nct:
            nr = (t1 - t0) // nct
            rows, cols = pl.ds(8 * r, 8 * nr), pl.ds(0, 128 * nct)
            t0 += nr * nct
        else:
            nc = min(nct - c, t1 - t0)
            rows, cols = pl.ds(8 * r, 8), pl.ds(128 * c, 128 * nc)
            t0 += nc
        out.append((src.at[rows, cols], dst.at[rows, cols]))
    return out


def _add_rows(stream, src, dst, r0, r1, small, bulk, even=False, extra=()):
    nct = src.shape[1] // 128
    t0, t1 = r0 // 8 * nct, r1 // 8 * nct
    if even:
        n = max(1, round((t1 - t0) / (small + bulk)))
        cuts = [t0 + (t1 - t0) * u // n for u in range(n + 1)]
    else:
        cuts = list(range(t0, t1, small + bulk)) + [t1]
    out = []
    for lo, hi in zip(cuts, cuts[1:]):
        s = small if hi - lo > small else 0
        unit = stream.add(_tile_copies(src, dst, lo, lo + s) + list(extra),
                          _tile_copies(src, dst, lo + s, hi))
        extra = ()
        out.append((hi // nct * 8, unit))
    return out


def _unit_for(ready, rows):
    return min(unit for (done, unit) in ready if done >= rows)


def _layernorm(x):
    m = jnp.mean(x, axis=-1, keepdims=True)
    d = x - m
    v = jnp.mean(d * d, axis=-1, keepdims=True)
    return d * lax.rsqrt(v + EPS)


def _body(x_hbm, c_hbm, wsp_hbm, bsp_hbm, k_hbm, v_hbm, wq_hbm, woT_hbm, win_hbm, woutT_hbm, wmod_hbm,
          o_ref,
          x_v, c_v, wsp_v, bsp_v, wmod_v, wq_v, k_v, v_v, woT_v, win_v, woutT_v, q_v, mod_v,
          sems, *, sk, w):
    st = _Stream(sems)
    small_inputs = [(c_hbm, c_v), (x_hbm, x_v), (wsp_hbm, wsp_v), (bsp_hbm, bsp_v)]
    u_wmod = _add_rows(st, wmod_hbm, wmod_v, 0, D, *UNIT, extra=small_inputs)
    u_wq = _add_rows(st, wq_hbm, wq_v, 0, D, *UNIT)
    u_wo = _add_rows(st, woT_hbm, woT_v, 0, D, *UNIT)
    u_k, u_v = [], []
    for j in range(HKV):
        window = pl.ds(sk - w, w)
        u_k.append(_add_rows(st, k_hbm.at[0, j, window, :], k_v.at[j], 0, w, *UNIT))
        u_v.append(_add_rows(st, v_hbm.at[0, j, window, :], v_v.at[j], 0, w, *UNIT))
    win_cuts = list(range(0, D, 128)) + [D]
    u_win = [_add_rows(st, win_hbm, win_v, r0, r1, *UNIT, even=True)[-1][1]
             for r0, r1 in zip(win_cuts, win_cuts[1:])]
    wout_cuts = [sum(WOUT_CUTS[:i]) for i in range(len(WOUT_CUTS) + 1)]
    u_wout = [_add_rows(st, woutT_hbm, woutT_v, r0, r1, 0, (r1 - r0) * FH)[-1][1]
              for r0, r1 in zip(wout_cuts, wout_cuts[1:])]
    st.pump()

    st.wait_through(u_wmod[0][1])
    cf = c_v[...].astype(F32)
    sc = (cf * jax.nn.sigmoid(cf)).astype(BF16)
    x = jnp.broadcast_to(x_v[0].astype(F32), (8, D))
    lnx = _layernorm(x)
    st.wait_through(u_wmod[-1][1])
    mod = jnp.dot(jnp.broadcast_to(sc, (8, D)), wmod_v[...], preferred_element_type=F32)
    for i in range(6):
        mod_v[i] = mod[:, i * D:(i + 1) * D]

    h = (lnx * (1.0 + mod_v[1]) + mod_v[0]).astype(BF16)
    st.wait_through(u_wq[-1][1])
    q = jnp.dot(h, wq_v[...], preferred_element_type=F32) * (DH ** -0.5)
    row = lax.broadcasted_iota(jnp.int32, (8, DH), 0)
    for j in range(HKV):
        q_v[j] = jnp.where(row == 0, q[:, 2 * j * DH:(2 * j + 1) * DH],
                           q[:, (2 * j + 1) * DH:(2 * j + 2) * DH])
    st.wait_through(u_wo[-1][1])

    attn = jnp.zeros((8, D), F32)
    chunks = [(r, r + KV_CHUNK) for r in range(0, w, KV_CHUNK)]
    for j in range(HKV):
        qj = q_v[j].astype(BF16)
        scores = []
        for r0, r1 in chunks:
            st.wait_through(_unit_for(u_k[j], r1))
            scores.append(lax.dot_general(qj, k_v[j, r0:r1, :], NT, preferred_element_type=F32))
        s = jnp.concatenate(scores, axis=1)
        e = jnp.exp(s - jnp.max(s, axis=-1, keepdims=True))
        denom = jnp.sum(e, axis=-1, keepdims=True)
        p = e.astype(BF16)
        acc = jnp.zeros((8, DH), F32)
        for r0, r1 in chunks:
            st.wait_through(_unit_for(u_v[j], r1))
            acc = acc + jnp.dot(p[:, r0:r1], v_v[j, r0:r1, :], preferred_element_type=F32)
        o = acc / denom
        o_pair = jnp.concatenate([jnp.broadcast_to(o[0:1, :], (8, DH)),
                                  jnp.broadcast_to(o[1:2, :], (8, DH))], axis=1).astype(BF16)
        attn = attn + lax.dot_general(o_pair, woT_v[:, 2 * DH * j:2 * DH * (j + 1)], NT,
                                      preferred_element_type=F32)

    x1 = x + mod_v[2] * attn
    h2 = (_layernorm(x1) * (1.0 + mod_v[4]) + mod_v[3]).astype(BF16)
    z = None
    for (r0, r1), unit in zip(zip(win_cuts, win_cuts[1:]), u_win):
        st.wait_through(unit)
        part = jnp.dot(h2[:, r0:r1], win_v[r0:r1, :], preferred_element_type=F32)
        z = part if z is None else z + part
    z = jax.nn.gelu(z, approximate=True)
    g = _layernorm(z[:, FH:]) * wsp_v[...].astype(F32) + bsp_v[...].astype(F32)
    y = (z[:, :FH] * g).astype(BF16)
    outs = []
    for (r0, r1), unit in zip(zip(wout_cuts, wout_cuts[1:]), u_wout):
        st.wait_through(unit)
        outs.append(lax.dot_general(y, woutT_v[r0:r1, :], NT, preferred_element_type=F32))
    x2 = x1 + mod_v[5] * jnp.concatenate(outs, axis=1)
    o_ref[...] = x2[0:1, :].astype(BF16)


def _kernel(*refs, **kwargs):
    pl.run_scoped(functools.partial(_body, *refs, **kwargs), pltpu.SemaphoreType.DMA((NSEM,)))


@jax.jit
def pallas_adaLN_cond__sliding_block_cached__mixer_gmlp__decode_kernel(
    A_x: jax.Array,
    A_k_cache: jax.Array,
    A_v_cache: jax.Array,
    A_wq: jax.Array,
    A_wo: jax.Array,
    B_x: jax.Array,
    B_w_in: jax.Array,
    B_w_sp: jax.Array,
    B_b_sp: jax.Array,
    B_w_out: jax.Array,
    c: jax.Array,
    w_mod: jax.Array,
):
    del B_x
    sk = A_k_cache.shape[2]
    w = min(4096, max(256, sk // 4))
    any_spec = pl.BlockSpec(memory_space=pl.ANY)
    out = pl.pallas_call(
        functools.partial(_kernel, sk=sk, w=w),
        out_shape=jax.ShapeDtypeStruct((1, D), BF16),
        in_specs=[any_spec] * 11,
        out_specs=pl.BlockSpec(memory_space=pltpu.VMEM),
        scratch_shapes=[
            pltpu.VMEM((1, 1, D), BF16),
            pltpu.VMEM((1, D), BF16),
            pltpu.VMEM((1, 1), BF16),
            pltpu.VMEM((1, 1), BF16),
            pltpu.VMEM((D, 6 * D), BF16),
            pltpu.VMEM((D, HQ * DH), BF16),
            pltpu.VMEM((HKV, w, DH), BF16),
            pltpu.VMEM((HKV, w, DH), BF16),
            pltpu.VMEM((D, HQ * DH), BF16),
            pltpu.VMEM((D, 2 * FH), BF16),
            pltpu.VMEM((D, FH), BF16),
            pltpu.VMEM((HKV, 8, DH), F32),
            pltpu.VMEM((6, 8, D), F32),
        ],
        compiler_params=pltpu.CompilerParams(vmem_limit_bytes=64 * 1024 * 1024),
    )(A_x, c, B_w_sp, B_b_sp.reshape(1, 1), A_k_cache, A_v_cache, A_wq, A_wo.T, B_w_in, B_w_out.T,
      w_mod)
    return out.reshape(1, 1, D)
```
